```python
import jax
import jax.numpy as jnp

def _softmax(x, axis=-1):
    return jax.nn.softmax(x, axis=axis)
def _gelu(x):
    return jax.nn.gelu(x, approximate=True)
def _silu(x):
    return jax.nn.silu(x)
def _sigmoid(x):
    return jax.nn.sigmoid(x)
def _layernorm(x, axis=-1, eps=1e-5):
    m = jnp.mean(x, axis=axis, keepdims=True)
    v = jnp.var(x, axis=axis, keepdims=True)
    return (x - m) / jnp.sqrt(v + eps)
def _scatter_add(tgt, idx, src, axis=0):
    return tgt.at[idx].add(src)
def _segment_sum(src, seg, n):
    return jax.ops.segment_sum(src, seg, n)
class _Rng:
    def __init__(self, key):
        self._k = key
    def _next(self):
        self._k, sub = jax.random.split(self._k)
        return sub
    def normal(self, shape):
        return jax.random.normal(self._next(), shape, dtype=jnp.bfloat16)
    def randint(self, lo, hi, shape):
        return jax.random.randint(self._next(), shape, lo, hi, dtype=jnp.int32)
    def uniform(self, shape, lo=0.0, hi=1.0):
        return jax.random.uniform(self._next(), shape, jnp.bfloat16, lo, hi)
    def permutation(self, n):
        return jax.random.permutation(self._next(), n)


kernel_name = 'recurrent_scan__mha_block_cached__moe_arch_mod__decode'

def setup_inputs():
    _rng = _Rng(jax.random.key(int.from_bytes(__import__("os").urandom(4), "little")))
    _w = (lambda a: (lambda t: t.astype(jnp.bfloat16) if jnp.issubdtype(t.dtype, jnp.floating) else t)(jnp.asarray(a)))
    def _A_setup():
        B, Sq, D = 2, 1, 512
        H, Sk, Dh = 32, 16384, 128
        return {
            "x": _w((lambda *s: _rng.normal(s) * 0.05)(B, Sq, D)),
            "k_cache": _w((lambda *s: _rng.normal(s) * 0.05)(B, H, Sk, Dh)),
            "v_cache": _w((lambda *s: _rng.normal(s) * 0.05)(B, H, Sk, Dh)),
            "wq": _w((lambda *s: _rng.normal(s) * 0.05)(D, H * Dh) * (D ** -0.5)),
            "wo": _w((lambda *s: _rng.normal(s) * 0.05)(H * Dh, D) * ((H * Dh) ** -0.5)),
        }
    _A_in = _A_setup()

    def _B_setup():
        B, S, D, F, C = 2, 1, 512, 1792, 1
        return {
            "x": _w((lambda *s: _rng.normal(s) * 0.05)(B, S, D)),
            "w_r": _w((lambda *s: _rng.normal(s) * 0.05)(D)),
            "w_gate": _w((lambda *s: _rng.normal(s) * 0.05)(D, F)),
            "w_up": _w((lambda *s: _rng.normal(s) * 0.05)(D, F)),
            "w_down": _w((lambda *s: _rng.normal(s) * 0.05)(F, D)),
        }
    _B_in = _B_setup()

    return {
        "A_x": _A_in["x"],
        "A_k_cache": _A_in["k_cache"],
        "A_v_cache": _A_in["v_cache"],
        "A_wq": _A_in["wq"],
        "A_wo": _A_in["wo"],
        "B_x": _B_in["x"],
        "B_w_r": _B_in["w_r"],
        "B_w_gate": _B_in["w_gate"],
        "B_w_up": _B_in["w_up"],
        "B_w_down": _B_in["w_down"],
    }

def reference(A_x, A_k_cache, A_v_cache, A_wq, A_wo, B_x, B_w_r, B_w_gate, B_w_up, B_w_down):
    def _A_ref(x, k_cache, v_cache, wq, wo):
        B, Sq, D = x.shape
        H, Dh = 32, 128
        q = (lambda x, *d: x.transpose(*d))((x @ wq).reshape(B, Sq, H, Dh), 0, 2, 1, 3)
        scores = jnp.einsum("bhqd,bhkd->bhqk", q, k_cache) * (Dh ** -0.5)
        p = _softmax(scores, axis=-1)
        o = jnp.einsum("bhqk,bhkd->bhqd", p, v_cache)
        return (lambda x, *d: x.transpose(*d))(o, 0, 2, 1, 3).reshape(B, Sq, H * Dh) @ wo

    def _B_ref(x, w_r, w_gate, w_up, w_down):
        B, S, D = x.shape
        C = 1
        r = x @ w_r
        idx = jnp.argsort(-r, axis=-1)[:, :C]
        idx_e = jnp.repeat(idx.reshape(B, C, 1), D, axis=2)
        x_sel = jnp.take_along_axis(x, idx_e, axis=1)
        g = _silu(x_sel @ w_gate)
        u = x_sel @ w_up
        y = (g * u) @ w_down
        r_sel = _sigmoid(jnp.take_along_axis(r, idx, axis=1))
        y = y * r_sel.reshape(B, C, 1)
        b_off = (jnp.arange(B) * S).reshape(B, 1)
        flat_idx = (idx + b_off).reshape(B * C)
        zero = (x * 0.0).reshape(B * S, D)
        upd = _scatter_add(zero, flat_idx, y.reshape(B * C, D), axis=0)
        return x + upd.reshape(B, S, D)

    x = A_x
    xn = _layernorm(x, axis=-1)
    s = _A_ref(xn, A_k_cache, A_v_cache, A_wq, A_wo)
    g = _silu(_B_ref(xn, B_w_r, B_w_gate, B_w_up, B_w_down))
    return x + s * g
```

```python
import jax
import jax.numpy as jnp
from jax import lax
import jax.experimental.pallas as pl
import jax.experimental.pallas.tpu as pltpu

B, H, S, DH, D, F = 2, 32, 16384, 128, 512, 1792
HG = 8
L = B * HG
G = H // HG
BLK = 256
P0 = 64
DEPTH = 2
NSLOT = 3
NJ = S // BLK
F32, BF16 = jnp.float32, jnp.bfloat16


def _kernel(x_hbm, k_hbm, v_hbm, wq_hbm, wo_hbm, wr_hbm, wg_hbm, wu_hbm, wd_hbm, o_ref,
            x_v, wr_v, wq_v, wo_v, wg_v, wu_v, wd_v, buf, q_scr, s_scr, p_scr, wsem, sems):
    def wcopy(src, dst, i):
        return pltpu.make_async_copy(src, dst, wsem.at[i])

    cx = wcopy(x_hbm, x_v, 0)
    cr = wcopy(wr_hbm, wr_v, 1)
    cq = wcopy(wq_hbm, wq_v, 2)
    cg = wcopy(wg_hbm, wg_v, 3)
    cu = wcopy(wu_hbm, wu_v, 4)
    cd = wcopy(wd_hbm, wd_v, 5)
    co = wcopy(wo_hbm, wo_v, 6)

    def start(a, g, j, r, slot):
        for off, rows, prio in ((0, P0, 0), (P0, BLK - P0, 1)):
            pltpu.make_async_copy(
                a.at[r // HG, g * HG + r % HG, pl.ds(j * BLK + off, rows)],
                buf.at[slot, r, pl.ds(off, rows)], sems.at[slot, r]).start(priority=prio)

    def wait(r, slot):
        pltpu.make_async_copy(buf.at[slot, r], buf.at[slot, r], sems.at[slot, r]).wait()

    cx.start(priority=0)
    cr.start(priority=0)
    for c in (cq, cg, cu, cd):
        c.start(priority=1)
    for d in range(DEPTH):
        for r in range(L):
            start(k_hbm, 0, d, r, d)

    cx.wait()
    x = x_v[...].astype(F32)
    mu = jnp.mean(x, axis=-1, keepdims=True)
    xc = x - mu
    var = jnp.mean(xc * xc, axis=-1, keepdims=True)
    xb = (xc / jnp.sqrt(var + 1e-5)).astype(BF16)
    cq.wait()
    q = jnp.dot(xb, wq_v[...], preferred_element_type=F32)
    for h in range(H):
        for b in range(B):
            row = (h // HG) * L + b * HG + h % HG
            q_scr[row:row + 1, :] = q[b:b + 1, h * DH:(h + 1) * DH]

    cr.wait()
    xf = xb.astype(F32)
    rr = jnp.sum(xf * wr_v[...].reshape(1, D).astype(F32), axis=-1, keepdims=True)
    cg.wait()
    gate = jnp.dot(xb, wg_v[...], preferred_element_type=F32)
    cu.wait()
    up = jnp.dot(xb, wu_v[...], preferred_element_type=F32)
    hid = (jax.nn.silu(gate) * up).astype(BF16)
    cd.wait()
    y = jnp.dot(hid, wd_v[...], preferred_element_type=F32) * jax.nn.sigmoid(rr)
    gmul = jax.nn.silu(xf + (xf * 0.0 + y))

    row8 = lax.broadcasted_iota(jnp.int32, (HG, BLK), 0)
    row8d = lax.broadcasted_iota(jnp.int32, (HG, DH), 0)

    def nxt(s, n=1):
        s = s + n
        return jnp.where(s >= NSLOT, s - NSLOT, s)

    def run(slot, compute, src):
        sslot = nxt(slot, DEPTH)
        for r in range(0, L, 2):
            wait(r, slot)
            wait(r + 1, slot)
            if src is not None:
                start(*src, r, sslot)
            compute(r, buf[slot, r])
            compute(r + 1, buf[slot, r + 1])
            if src is not None:
                start(*src, r + 1, sslot)

    def k_phase(g, slot):
        q16 = q_scr[pl.ds(pl.multiple_of(g * L, L), L), :]
        qs = [q16[b * HG:(b + 1) * HG].astype(BF16) for b in range(B)]

        def step(j, carry, src):
            m, slot = carry
            sc = [None] * B

            def compute(r, kt):
                b, i = divmod(r, HG)
                s = lax.dot_general(qs[b], kt, (((1,), (1,)), ((), ())), preferred_element_type=F32)
                sc[b] = s if sc[b] is None else jnp.where(row8 == i, s, sc[b])

            run(slot, compute, src)
            s = jnp.concatenate(sc, axis=0) * (DH ** -0.5)
            s_scr[j] = s
            return jnp.maximum(m, s), nxt(slot)

        c = (jnp.full((L, BLK), -jnp.inf, F32), slot)
        c = lax.fori_loop(0, NJ - DEPTH, lambda j, c: step(j, c, (k_hbm, g, j + DEPTH)), c)
        m, slot = lax.fori_loop(NJ - DEPTH, NJ, lambda j, c: step(j, c, (v_hbm, g, j + DEPTH - NJ)), c)
        m = jnp.max(m, axis=-1, keepdims=True)

        def pbody(j, l):
            p = jnp.exp(s_scr[j] - m)
            p_scr[j] = p.astype(BF16)
            return l + p

        l = lax.fori_loop(0, NJ, pbody, jnp.zeros((L, BLK), F32), unroll=8)
        return jnp.sum(l, axis=-1, keepdims=True), slot

    def v_phase(g, slot, last):
        def step(j, carry, src):
            acc, slot = carry
            p = p_scr[j]
            pb = [p[b * HG:(b + 1) * HG] for b in range(B)]
            acc = list(acc)

            def compute(r, vt):
                b, i = divmod(r, HG)
                o = jnp.dot(pb[b], vt, preferred_element_type=F32)
                acc[b] = acc[b] + jnp.where(row8d == i, o, 0.0)

            run(slot, compute, src)
            return tuple(acc), nxt(slot)

        c = (tuple(jnp.zeros((HG, DH), F32) for _ in range(B)), slot)
        c = lax.fori_loop(0, NJ - DEPTH, lambda j, c: step(j, c, (v_hbm, g, j + DEPTH)), c)
        c = lax.fori_loop(
            NJ - DEPTH, NJ,
            lambda j, c: step(j, c, None if last else (k_hbm, g + 1, j + DEPTH - NJ)), c)
        return jnp.concatenate(c[0], axis=0), c[1]

    def group(g, carry, last, first):
        s_acc, slot = carry
        l, slot = k_phase(g, slot)
        if first:
            co.start(priority=1)
        o, slot = v_phase(g, slot, last)
        o = o / l
        if first:
            co.wait()
        of = jnp.concatenate(
            [jnp.concatenate([o[b * HG + i:b * HG + i + 1] for b in range(B)], axis=0) for i in range(HG)],
            axis=1).astype(BF16)
        w = wo_v[pl.ds(pl.multiple_of(g * HG * DH, HG * DH), HG * DH), :]
        return s_acc + jnp.dot(of, w, preferred_element_type=F32), slot

    c = group(0, (jnp.zeros((B, D), F32), jnp.int32(0)), False, True)
    c = lax.fori_loop(1, G - 1, lambda g, c: group(g, c, False, False), c)
    s_acc, _ = group(G - 1, c, True, False)
    o_ref[...] = (x + s_acc * gmul).astype(o_ref.dtype)


@jax.jit
def pallas_recurrent_scan__mha_block_cached__moe_arch_mod__decode_kernel(
    A_x: jax.Array,
    A_k_cache: jax.Array,
    A_v_cache: jax.Array,
    A_wq: jax.Array,
    A_wo: jax.Array,
    B_x: jax.Array,
    B_w_r: jax.Array,
    B_w_gate: jax.Array,
    B_w_up: jax.Array,
    B_w_down: jax.Array,
):
    del B_x
    any_spec = pl.BlockSpec(memory_space=pl.ANY)
    out = pl.pallas_call(
        _kernel,
        out_shape=jax.ShapeDtypeStruct((B, D), A_x.dtype),
        in_specs=[any_spec] * 9,
        out_specs=pl.BlockSpec(memory_space=pltpu.VMEM),
        scratch_shapes=[
            pltpu.VMEM((B, D), BF16), pltpu.VMEM((D,), BF16),
            pltpu.VMEM((D, H * DH), BF16), pltpu.VMEM((H * DH, D), BF16),
            pltpu.VMEM((D, F), BF16), pltpu.VMEM((D, F), BF16), pltpu.VMEM((F, D), BF16),
            pltpu.VMEM((NSLOT, L, BLK, DH), BF16),
            pltpu.VMEM((G * L, DH), F32),
            pltpu.VMEM((NJ, L, BLK), F32), pltpu.VMEM((NJ, L, BLK), BF16),
            pltpu.SemaphoreType.DMA((7,)), pltpu.SemaphoreType.DMA((NSLOT, L)),
        ],
        compiler_params=pltpu.CompilerParams(vmem_limit_bytes=64 * 1024 * 1024),
    )(A_x.reshape(B, D), A_k_cache, A_v_cache, A_wq, A_wo, B_w_r, B_w_gate, B_w_up, B_w_down)
    return out.reshape(B, 1, D)
```

```python
import jax
import jax.numpy as jnp
from jax import lax
import jax.experimental.pallas as pl
import jax.experimental.pallas.tpu as pltpu

B, H, S, DH, D, F = 2, 32, 16384, 128, 512, 1792
HG = 8
L = B * HG
G = H // HG
GW = HG * DH
BLK = 256
P0 = 64
SHIFT = 128
DEPTH = 2
NSLOT = 3
NJ = S // BLK
F32, BF16 = jnp.float32, jnp.bfloat16


def _kernel(x_hbm, k_hbm, v_hbm, wq_hbm, wo_hbm, wr_hbm, wg_hbm, wu_hbm, wd_hbm, o_ref,
            x_v, wr_v, wq_v, wo_v, wg_v, wu_v, wd_v, buf,
            q_scr, s_scr, p_scr, acc_scr, h_scr, y_scr, wsem, sems):
    cp = pltpu.make_async_copy

    def start(a, g, j, may_wrap, r, slot):
        if may_wrap:
            lo = pl.multiple_of(jnp.where(j == 0, S - SHIFT, j * BLK - SHIFT), SHIFT)
            pieces = ((lo, 0, P0, 0), (lo + P0, P0, SHIFT - P0, 1), (j * BLK, SHIFT, BLK - SHIFT, 1))
        else:
            lo = j * BLK - SHIFT
            pieces = ((lo, 0, P0, 0), (lo + P0, P0, BLK - P0, 1))
        for src, dst, rows, prio in pieces:
            cp(a.at[r // HG, g * HG + r % HG, pl.ds(src, rows)],
               buf.at[slot, r, pl.ds(dst, rows)], sems.at[slot, r]).start(priority=prio)

    def wait_all(ref, sem):
        cp(ref, ref, sem).wait()

    cp(x_hbm, x_v, wsem.at[0]).start(priority=0)
    cp(wq_hbm.at[:, pl.ds(0, GW)], wq_v, wsem.at[2]).start(priority=0)
    cp(wr_hbm, wr_v, wsem.at[1]).start(priority=0)

    def prologue(d, c):
        for r in range(L):
            start(k_hbm, 0, d, True, r, d)
        return c

    lax.fori_loop(0, DEPTH, prologue, 0)

    wait_all(x_v, wsem.at[0])
    x = x_v[...].astype(F32)
    mu = jnp.mean(x, axis=-1, keepdims=True)
    xc = x - mu
    var = jnp.mean(xc * xc, axis=-1, keepdims=True)
    xb = (xc / jnp.sqrt(var + 1e-5)).astype(BF16)
    wait_all(wr_v, wsem.at[1])

    row_s = lax.broadcasted_iota(jnp.int32, (HG, BLK), 0)
    row_o = lax.broadcasted_iota(jnp.int32, (HG, DH), 0)

    def nxt(s, n=1):
        s = s + n
        return jnp.where(s >= NSLOT, s - NSLOT, s)

    def run(slot, compute, src):
        sslot = nxt(slot, DEPTH)
        for r in range(0, L, 2):
            wait_all(buf.at[slot, r], sems.at[slot, r])
            wait_all(buf.at[slot, r + 1], sems.at[slot, r + 1])
            if src is not None:
                start(*src, r, sslot)
            compute(r, buf[slot, r])
            compute(r + 1, buf[slot, r + 1])
            if src is not None:
                start(*src, r + 1, sslot)

    def k_weights(g, j):
        @pl.when(j < GW // 32)
        def _():
            cp(wo_hbm.at[pl.ds(pl.multiple_of(g * GW + j * 32, 32), 32)],
               wo_v.at[pl.ds(pl.multiple_of(j * 32, 32), 32)], wsem.at[3]).start(priority=1)

        j0 = NJ - DEPTH - D // 16

        @pl.when(jnp.logical_and(j >= j0, g < G - 1))
        def _():
            rows = pl.ds(pl.multiple_of((j - j0) * 16, 16), 16)
            cols = pl.ds(pl.multiple_of((g + 1) * GW, GW), GW)
            cp(wq_hbm.at[rows, cols], wq_v.at[rows], wsem.at[2]).start(priority=1)

    def v_weights(g, j):
        for gg, w_hbm, w_v, nr in ((0, wg_hbm, wg_v, 16), (1, wu_hbm, wu_v, 16), (2, wd_hbm, wd_v, 64)):
            @pl.when(jnp.logical_and(j < w_v.shape[0] // nr, g == gg))
            def _():
                rows = pl.ds(pl.multiple_of(j * nr, nr), nr)
                cp(w_hbm.at[rows], w_v.at[rows], wsem.at[4 + gg]).start(priority=1)

    def k_phase(g, slot):
        wait_all(wq_v, wsem.at[2])
        q = jnp.dot(xb, wq_v[...], preferred_element_type=F32)
        for b in range(B):
            for h in range(HG):
                q_scr[b * HG + h:b * HG + h + 1, :] = q[b:b + 1, h * DH:(h + 1) * DH]
        qs = [q_scr[b * HG:(b + 1) * HG].astype(BF16) for b in range(B)]

        def step(j, carry, src):
            m, slot = carry
            sc = [None] * B

            def compute(r, kt):
                b, i = divmod(r, HG)
                s = lax.dot_general(qs[b], kt, (((1,), (1,)), ((), ())), preferred_element_type=F32)
                sc[b] = s if sc[b] is None else jnp.where(row_s == i, s, sc[b])

            run(slot, compute, src)
            s = jnp.concatenate(sc, axis=0) * (DH ** -0.5)
            s_scr[j] = s
            return jnp.maximum(m, s), nxt(slot)

        def main(j, c):
            k_weights(g, j)
            return step(j, c, (k_hbm, g, j + DEPTH, False))

        c = (jnp.full((L, BLK), -jnp.inf, F32), slot)
        c = lax.fori_loop(0, NJ - DEPTH, main, c)
        m, slot = lax.fori_loop(NJ - DEPTH, NJ, lambda j, c: step(j, c, (v_hbm, g, j + DEPTH - NJ, True)), c)
        m = jnp.max(m, axis=-1, keepdims=True)

        def pbody(j, l):
            p = jnp.exp(s_scr[j] - m)
            p_scr[j] = p.astype(BF16)
            return l + p

        l = lax.fori_loop(0, NJ, pbody, jnp.zeros((L, BLK), F32), unroll=8)
        return jnp.sum(l, axis=-1, keepdims=True), slot

    def v_phase(g, slot):
        def step(j, carry, src):
            acc, slot = carry
            p = p_scr[j]
            pb = [p[b * HG:(b + 1) * HG] for b in range(B)]
            acc = list(acc)

            def compute(r, vt):
                b, i = divmod(r, HG)
                o = jnp.dot(pb[b], vt, preferred_element_type=F32)
                acc[b] = acc[b] + jnp.where(row_o == i, o, 0.0)

            run(slot, compute, src)
            return tuple(acc), nxt(slot)

        def main(j, c):
            v_weights(g, j)
            return step(j, c, (v_hbm, g, j + DEPTH, False))

        c = (tuple(jnp.zeros((HG, DH), F32) for _ in range(B)), slot)
        c = lax.fori_loop(0, NJ - DEPTH, main, c)

        def tail(last):
            acc, _ = lax.fori_loop(
                NJ - DEPTH, NJ,
                lambda j, c: step(j, c, None if last else (k_hbm, g + 1, j + DEPTH - NJ, True)), c)
            acc_scr[...] = jnp.concatenate(acc, axis=0)

        pl.when(g < G - 1)(lambda: tail(False))
        pl.when(g == G - 1)(lambda: tail(True))
        return acc_scr[...], nxt(c[1], DEPTH)

    def group(g, carry):
        s_acc, slot = carry
        l, slot = k_phase(g, slot)
        wait_all(wo_v, wsem.at[3])
        o, slot = v_phase(g, slot)
        o = o / l
        of = jnp.concatenate(
            [jnp.concatenate([o[b * HG + i:b * HG + i + 1] for b in range(B)], axis=0) for i in range(HG)],
            axis=1).astype(BF16)
        s_acc = s_acc + jnp.dot(of, wo_v[...], preferred_element_type=F32)

        @pl.when(g == 0)
        def _():
            wait_all(wg_v, wsem.at[4])
            h_scr[...] = jax.nn.silu(jnp.dot(xb, wg_v[...], preferred_element_type=F32))

        @pl.when(g == 1)
        def _():
            wait_all(wu_v, wsem.at[5])
            h_scr[...] = h_scr[...] * jnp.dot(xb, wu_v[...], preferred_element_type=F32)

        @pl.when(g == 2)
        def _():
            wait_all(wd_v, wsem.at[6])
            xf = xb.astype(F32)
            rr = jnp.sum(xf * wr_v[...].reshape(1, D).astype(F32), axis=-1, keepdims=True)
            y = jnp.dot(h_scr[...].astype(BF16), wd_v[...], preferred_element_type=F32) * jax.nn.sigmoid(rr)
            y_scr[...] = jax.nn.silu(xf + (xf * 0.0 + y))

        return s_acc, slot

    s_acc, _ = lax.fori_loop(0, G, group, (jnp.zeros((B, D), F32), jnp.int32(0)))
    o_ref[...] = (x + s_acc * y_scr[...]).astype(o_ref.dtype)


@jax.jit
def pallas_recurrent_scan__mha_block_cached__moe_arch_mod__decode_kernel(
    A_x: jax.Array,
    A_k_cache: jax.Array,
    A_v_cache: jax.Array,
    A_wq: jax.Array,
    A_wo: jax.Array,
    B_x: jax.Array,
    B_w_r: jax.Array,
    B_w_gate: jax.Array,
    B_w_up: jax.Array,
    B_w_down: jax.Array,
):
    del B_x
    any_spec = pl.BlockSpec(memory_space=pl.ANY)
    out = pl.pallas_call(
        _kernel,
        out_shape=jax.ShapeDtypeStruct((B, D), A_x.dtype),
        in_specs=[any_spec] * 9,
        out_specs=pl.BlockSpec(memory_space=pltpu.VMEM),
        scratch_shapes=[
            pltpu.VMEM((B, D), BF16), pltpu.VMEM((D,), BF16),
            pltpu.VMEM((D, GW), BF16), pltpu.VMEM((GW, D), BF16),
            pltpu.VMEM((D, F), BF16), pltpu.VMEM((D, F), BF16), pltpu.VMEM((F, D), BF16),
            pltpu.VMEM((NSLOT, L, BLK, DH), BF16),
            pltpu.VMEM((L, DH), F32),
            pltpu.VMEM((NJ, L, BLK), F32), pltpu.VMEM((NJ, L, BLK), BF16),
            pltpu.VMEM((L, DH), F32), pltpu.VMEM((B, F), F32), pltpu.VMEM((B, D), F32),
            pltpu.SemaphoreType.DMA((7,)), pltpu.SemaphoreType.DMA((NSLOT, L)),
        ],
        compiler_params=pltpu.CompilerParams(vmem_limit_bytes=64 * 1024 * 1024),
    )(A_x.reshape(B, D), A_k_cache, A_v_cache, A_wq, A_wo, B_w_r, B_w_gate, B_w_up, B_w_down)
    return out.reshape(B, 1, D)
```
